```python
import os as _os
_os.environ.setdefault("JAX_PLATFORMS", "cpu")
import jax
import jax.numpy as jnp

def _softmax(x, axis=-1):
    return jax.nn.softmax(x, axis=axis)
def _gelu(x):
    return jax.nn.gelu(x, approximate=True)
def _silu(x):
    return jax.nn.silu(x)
def _sigmoid(x):
    return jax.nn.sigmoid(x)
def _layernorm(x, axis=-1, eps=1e-5):
    m = jnp.mean(x, axis=axis, keepdims=True)
    v = jnp.var(x, axis=axis, keepdims=True)
    return (x - m) / jnp.sqrt(v + eps)
def _scatter_add(tgt, idx, src, axis=0):
    return tgt.at[idx].add(src)
def _segment_sum(src, seg, n):
    return jax.ops.segment_sum(src, seg, n)
class _Rng:
    def __init__(self, key):
        self._k = key
    def _next(self):
        self._k, sub = jax.random.split(self._k)
        return sub
    def normal(self, shape):
        return jax.random.normal(self._next(), shape, dtype=jnp.bfloat16)
    def randint(self, lo, hi, shape):
        return jax.random.randint(self._next(), shape, lo, hi, dtype=jnp.int32)
    def uniform(self, shape, lo=0.0, hi=1.0):
        return jax.random.uniform(self._next(), shape, jnp.bfloat16, lo, hi)
    def permutation(self, n):
        return jax.random.permutation(self._next(), n)


kernel_name = 'concat_heads__mha_block_cached__mha_block_cached__near_ridge'

def setup_inputs():
    _rng = _Rng(jax.random.key(int.from_bytes(__import__("os").urandom(4), "little")))
    _w = (lambda a: (lambda t: t.astype(jnp.bfloat16) if jnp.issubdtype(t.dtype, jnp.floating) else t)(jnp.asarray(a)))
    def _A_setup():
        B, Sq, D = 16, 32, 1024
        H, Sk, Dh = 32, 32, 128
        return {
            "x": _w((lambda *s: _rng.normal(s) * 0.8)(B, Sq, D)),
            "k_cache": _w((lambda *s: _rng.normal(s) * 0.8)(B, H, Sk, Dh)),
            "v_cache": _w((lambda *s: _rng.normal(s) * 0.05)(B, H, Sk, Dh)),
            "wq": _w((lambda *s: _rng.normal(s) * 0.8)(D, H * Dh) * (D ** -0.5)),
            "wo": _w((lambda *s: _rng.normal(s) * 0.05)(H * Dh, D) * ((H * Dh) ** -0.5)),
        }
    _A_in = _A_setup()

    def _B_setup():
        B, Sq, D = 16, 32, 1024
        H, Sk, Dh = 32, 32, 128
        return {
            "x": _w((lambda *s: _rng.normal(s) * 0.8)(B, Sq, D)),
            "k_cache": _w((lambda *s: _rng.normal(s) * 0.8)(B, H, Sk, Dh)),
            "v_cache": _w((lambda *s: _rng.normal(s) * 0.05)(B, H, Sk, Dh)),
            "wq": _w((lambda *s: _rng.normal(s) * 0.8)(D, H * Dh) * (D ** -0.5)),
            "wo": _w((lambda *s: _rng.normal(s) * 0.05)(H * Dh, D) * ((H * Dh) ** -0.5)),
        }
    _B_in = _B_setup()

    return {
        "A_x": _A_in["x"],
        "A_k_cache": _A_in["k_cache"],
        "A_v_cache": _A_in["v_cache"],
        "A_wq": _A_in["wq"],
        "A_wo": _A_in["wo"],
        "B_x": _B_in["x"],
        "B_k_cache": _B_in["k_cache"],
        "B_v_cache": _B_in["v_cache"],
        "B_wq": _B_in["wq"],
        "B_wo": _B_in["wo"],
    }

def reference(A_x, A_k_cache, A_v_cache, A_wq, A_wo, B_x, B_k_cache, B_v_cache, B_wq, B_wo):
    def _A_ref(x, k_cache, v_cache, wq, wo):
        B, Sq, D = x.shape
        H, Dh = 32, 128
        q = (lambda x, *d: x.transpose(*d))((x @ wq).reshape(B, Sq, H, Dh), 0, 2, 1, 3)
        scores = jnp.einsum("bhqd,bhkd->bhqk", q, k_cache) * (Dh ** -0.5)
        p = _softmax(scores, axis=-1)
        o = jnp.einsum("bhqk,bhkd->bhqd", p, v_cache)
        return (lambda x, *d: x.transpose(*d))(o, 0, 2, 1, 3).reshape(B, Sq, H * Dh) @ wo

    def _B_ref(x, k_cache, v_cache, wq, wo):
        B, Sq, D = x.shape
        H, Dh = 32, 128
        q = (lambda x, *d: x.transpose(*d))((x @ wq).reshape(B, Sq, H, Dh), 0, 2, 1, 3)
        scores = jnp.einsum("bhqd,bhkd->bhqk", q, k_cache) * (Dh ** -0.5)
        p = _softmax(scores, axis=-1)
        o = jnp.einsum("bhqk,bhkd->bhqd", p, v_cache)
        return (lambda x, *d: x.transpose(*d))(o, 0, 2, 1, 3).reshape(B, Sq, H * Dh) @ wo

    a = _A_ref(A_x, A_k_cache, A_v_cache, A_wq, A_wo)
    b = _B_ref(B_x, B_k_cache, B_v_cache, B_wq, B_wo)
    return jnp.concatenate([a, b], axis=-1)
```

```python
import functools
import jax
import jax.numpy as jnp
from jax import lax
import jax.experimental.pallas as pl
import jax.experimental.pallas.tpu as pltpu

B, SQ, D = 16, 32, 1024
H, SK, DH = 32, 32, 128
M = B * SQ
BG = 128 // SQ
NG = B // BG
LOG2E = 1.4426950408889634
F32 = jnp.float32
BF16 = jnp.bfloat16
G = 4
N = G * DH
GPB = H // G
NJ = 2 * GPB
CN = 128
NC = D // CN
LA = 2
NQ = 4


def substep_ops(ja, jb, jc):
    ops = []
    cs = list(range(NC)) if jc is not None else []
    for h in range(G):
        if jb is not None:
            ops.append(('B', jb, h))
        if cs:
            ops.append(('C', jc, cs.pop(0)))
        if ja is not None:
            ops.append(('A', ja, h))
        if jb is not None:
            ops.append(('D', jb, h))
        if cs:
            ops.append(('C', jc, cs.pop(0)))
    assert not cs
    return ops


def default_plan(loops, ramp_kind=0):
    A = lambda g: ('A', g // G, g % G)
    Bo = lambda g: ('B', g // G, g % G)
    Do = lambda g: ('D', g // G, g % G)
    if ramp_kind == 0:
        ramp = [
            [A(0)],
            [A(1), A(2)],
            [A(3), A(4), A(5), A(6)],
            [A(7)] + substep_ops(2, 0, None),
        ]
    elif ramp_kind == 1:
        ramp = [
            [A(0)],
            [A(1), A(2)],
            [A(3), A(4), A(5), A(6)],
            [Bo(0), A(7), Do(0), Bo(1), A(8), Do(1), Bo(2), A(9), Do(2), Bo(3), A(10), Do(3), A(11)],
        ]
    j0 = loops[0][0]
    j1 = loops[-1][1]
    for j in range(1, j0):
        ramp.append(substep_ops(j + LA, j, j - 1))
    tail = []
    for j in range(j1, NJ):
        tail += substep_ops(j + LA if j + LA < NJ else None, j, j - 1)
    tail += [('F', NJ - 1, n) for n in range(NC)]
    return ramp, loops, [tail]


def _make(loops=((1, 3, 1), (3, 13, 2)), ramp_kind=1, WAITALL=False, plan=None):
    ramp, loops, tail = plan or default_plan(loops, ramp_kind)

    have = set()
    dma = []

    def need(ops, sem):
        items = []
        for op in ops:
            kind, j, i = op
            key = {'A': 'wq', 'B': 'k', 'D': 'v', 'C': 'wo', 'F': 'wo'}[kind]
            if kind == 'A' and ('x', j // GPB) not in have:
                have.add(('x', j // GPB))
                items.append(('x', j // GPB, 0))
            if (key, j, i) not in have:
                have.add((key, j, i))
                items.append((key, j, i))
        out = []
        for key, j, i in items:
            for o in out:
                if o[0] == key and o[1] == j and o[3] == i:
                    o[3] = i + 1
                    break
            else:
                out.append([key, j, i, i + 1])
        return [(sem, *o) for o in out]

    sem = 0
    ramp_waits = []
    for ph in ramp:
        d = need(ph, sem); dma += d; ramp_waits.append(d); sem += 1
    SEM_XB = sem; sem += 1
    loop_info = []
    for (j0, j1, U) in loops:
        assert (j1 - j0) % U == 0
        n_iter = (j1 - j0) // U
        sem0 = sem
        xb_iter = None
        for it in range(n_iter):
            ops = []
            for u in range(U):
                j = j0 + it * U + u
                ops += substep_ops(j + LA, j, j - 1)
            d = need(ops, sem)
            d2 = []
            for e in d:
                if e[1] == 'x':
                    xb_iter = it
                    d2.append((SEM_XB, *e[1:]))
                else:
                    assert e[3] == 0 and e[4] == (NC if e[1] == 'wo' else G), e
                    d2.append(e)
            dma += d2
            sem += 1
        loop_info.append((j0, U, n_iter, sem0, xb_iter))
    tail_waits = []
    for ph in tail:
        d = need(ph, sem); dma += d; tail_waits.append(d); sem += 1
    SEM_OUT = sem; sem += 1
    NSEM = sem

    def kernel(ax, ak, av, awq, awo, bx, bk, bv, bwq, bwo, out_hbm,
               x_buf, wq_buf, wo_buf, k_buf, v_buf, acc, q_buf, o_buf, o_stage, sems):
        srcs = ((ax, ak, av, awq, awo), (bx, bk, bv, bwq, bwo))

        def copy(sem, kind, j, lo, hi, static=True):
            br, s = divmod(j, GPB) if static else (0, 0)
            sx, sk, sv, swq, swo = srcs[br]
            if kind == 'x':
                return pltpu.make_async_copy(srcs[j][0], x_buf.at[j], sems.at[sem])
            if kind == 'wq':
                return pltpu.make_async_copy(swq.at[:, pl.ds(s * N + lo * DH, (hi - lo) * DH)],
                                             wq_buf.at[j, :, pl.ds(lo * DH, (hi - lo) * DH)], sems.at[sem])
            if kind == 'wo':
                return pltpu.make_async_copy(swo.at[pl.ds(s * N, N), pl.ds(lo * CN, (hi - lo) * CN)],
                                             wo_buf.at[j, :, pl.ds(lo * CN, (hi - lo) * CN)], sems.at[sem])
            src, buf = (sk, k_buf) if kind == 'k' else (sv, v_buf)
            return pltpu.make_async_copy(src.at[:, pl.ds(s * G + lo, hi - lo)],
                                         buf.at[j, :, pl.ds(lo, hi - lo)], sems.at[sem])

        for e in dma:
            copy(*e).start()

        acc[...] = jnp.zeros_like(acc)

        row_b = lax.broadcasted_iota(jnp.int32, (128, 128), 0) // SQ
        col_b = lax.broadcasted_iota(jnp.int32, (128, 128), 1) // SK
        c = (DH ** -0.5) * LOG2E
        out_copies = []

        def run_ops(ops, base):
            mask = row_b == col_b
            xs, os_, es = {}, {}, {}
            static = isinstance(base, int)
            for op in ops:
                kind, jr, i = op
                j = base + jr
                if kind == 'A':
                    xkey = j // GPB if static else jr
                    if xkey not in xs:
                        xs[xkey] = x_buf[j // GPB]
                    q = jnp.dot(xs[xkey], wq_buf[j, :, i * DH:(i + 1) * DH],
                                preferred_element_type=F32).astype(BF16)
                    q_buf[j % NQ, :, i * DH:(i + 1) * DH] = q
                elif kind == 'B':
                    ss = []
                    for g in range(NG):
                        qg = q_buf[j % NQ, g * 128:(g + 1) * 128, i * DH:(i + 1) * DH]
                        kg = k_buf[j, g * BG:(g + 1) * BG, i].reshape(128, DH)
                        ss.append(lax.dot_general(qg, kg, (((1,), (1,)), ((), ())),
                                                  preferred_element_type=F32))
                    ee = []
                    for g in range(NG):
                        s = jnp.where(mask, ss[g], -jnp.inf)
                        m = jnp.max(s, axis=-1, keepdims=True)
                        ex = jnp.exp2((s - m) * c)
                        l = jnp.sum(ex, axis=-1, keepdims=True)
                        ee.append((ex.astype(BF16), pl.reciprocal(l, approx=True)))
                    es[(jr, i)] = ee
                elif kind == 'D':
                    ee = es.pop((jr, i))
                    for g in range(NG):
                        vg = v_buf[j, g * BG:(g + 1) * BG, i].reshape(128, DH)
                        o = jnp.dot(ee[g][0], vg, preferred_element_type=F32) * ee[g][1]
                        o_buf[g * 128:(g + 1) * 128, i * DH:(i + 1) * DH] = o.astype(BF16)
                else:
                    if jr not in os_:
                        os_[jr] = o_buf[...]
                    cols = slice(i * CN, (i + 1) * CN)
                    r = jnp.dot(os_[jr], wo_buf[j, :, cols], preferred_element_type=F32)
                    if kind == 'C':
                        acc[j // GPB, :, cols] += r
                    else:
                        for br in range(2):
                            val = acc[br, :, cols] + r if br == 1 else acc[br, :, cols]
                            o_stage[br, :, cols] = val.astype(BF16)
                            cp = pltpu.make_async_copy(
                                o_stage.at[br, :, pl.ds(i * CN, CN)],
                                out_hbm.at[:, pl.ds(br * D + i * CN, CN)], sems.at[SEM_OUT])
                            cp.start()
                            out_copies.append(cp)
            assert not es

        if WAITALL:
            for e in dma:
                copy(*e).wait()
        for ph, w in zip(ramp, ramp_waits):
            if not WAITALL:
                for e in w:
                    copy(*e).wait()
            run_ops(ph, 0)

        for (j0, U, n_iter, sem0, xb_iter) in loop_info:
            loop_ops = []
            for u in range(U):
                loop_ops += substep_ops(u + LA, u, u - 1)

            def loop_body(it, carry, j0=j0, U=U, sem0=sem0, xb_iter=xb_iter, loop_ops=loop_ops):
                jb = j0 + it * U
                if not WAITALL:
                    if xb_iter is not None:
                        @pl.when(it == xb_iter)
                        def _():
                            copy(SEM_XB, 'x', 1, 0, 1).wait()
                    for u in range(U):
                        s = sem0 + it
                        copy(s, 'wq', jb + u + LA, 0, G, static=False).wait()
                        copy(s, 'k', jb + u, 0, G, static=False).wait()
                        copy(s, 'v', jb + u, 0, G, static=False).wait()
                        copy(s, 'wo', jb + u - 1, 0, NC, static=False).wait()
                run_ops(loop_ops, jb)
                return carry

            lax.fori_loop(0, n_iter, loop_body, 0)

        for ph, w in zip(tail, tail_waits):
            if not WAITALL:
                for e in w:
                    copy(*e).wait()
            run_ops(ph, 0)
        for cp in out_copies:
            cp.wait()

    def fn(A_x, A_k_cache, A_v_cache, A_wq, A_wo, B_x, B_k_cache, B_v_cache, B_wq, B_wo):
        any_spec = pl.BlockSpec(memory_space=pl.ANY)
        out = pl.pallas_call(
            kernel,
            in_specs=[any_spec] * 10,
            out_specs=any_spec,
            out_shape=jax.ShapeDtypeStruct((M, 2 * D), BF16),
            scratch_shapes=[
                pltpu.VMEM((2, M, D), BF16),
                pltpu.VMEM((NJ, D, N), BF16),
                pltpu.VMEM((NJ, N, D), BF16),
                pltpu.VMEM((NJ, B, G, SK, DH), BF16),
                pltpu.VMEM((NJ, B, G, SK, DH), BF16),
                pltpu.VMEM((2, M, D), F32),
                pltpu.VMEM((NQ, M, N), BF16),
                pltpu.VMEM((M, N), BF16),
                pltpu.VMEM((2, M, D), BF16),
                pltpu.SemaphoreType.DMA((NSEM,)),
            ],
            compiler_params=pltpu.CompilerParams(
                vmem_limit_bytes=100 * 1024 * 1024,
            ),
        )(A_x.reshape(M, D), A_k_cache, A_v_cache, A_wq, A_wo,
          B_x.reshape(M, D), B_k_cache, B_v_cache, B_wq, B_wo)
        return out.reshape(B, SQ, 2 * D)
    return fn


pallas_concat_heads__mha_block_cached__mha_block_cached__near_ridge_kernel = jax.jit(_make())
```

```python
import jax
import jax.numpy as jnp
from jax import lax
import jax.experimental.pallas as pl
import jax.experimental.pallas.tpu as pltpu

B, SQ, D = 16, 32, 1024
H, SK, DH = 32, 32, 128
M = B * SQ
BG = 128 // SQ
NG = B // BG
G = 4
N = G * DH
GPB = H // G
NJ = 2 * GPB
CN = 128
NC = D // CN
NQ = 4
LA = 3
XB = 4
XR = M // XB
PAD = 128
LAST_SPLIT = 8
F32 = jnp.float32
BF16 = jnp.bfloat16
EXP2_SCALE = (DH ** -0.5) * 1.4426950408889634

ORDER_FULL = 'P0 P1 P2 P3 A3 B0 C0 B1 C1 B2 C2 B3 A0 D0 A1 C3 D1 A2 C4 D2 C5 C6 C7 D3'
ORDER_NO_A = 'P0 P1 P2 P3 C0 B0 C1 C2 D0 B1 C3 C4 D1 B2 C5 B3 C6 D2 C7 D3'
RAMP = ['a0:02 a1:02', 'a0:24 a1:24', 'A2 A3', 'A4 A5 A6 A7', 'A8 A9 A10 A11',
        'P0 P1 P2 P3 A12 B0 B1 B2 B3 A13 D0 A14 D1 D2 A15 D3']
LOOPS = ((1, 3, 1, (32, 48, 48, 48), 5),
         (3, 13, 2, (32, 48, 48, 48, 48, 48, 48, 48), 4))
OFF_RAMP = (32, 16, 16, 32)
OFF_TAIL = (16, 32, 32, 16) * 3
PACE = 5
OUT_STARTS = (2, 4, 6, 7)


def _step_ops(ja, jb, jc):
    grp = {'A': ja, 'B': jb, 'D': jb, 'P': jb, 'C': jc}
    return [(t[0], grp[t[0]], int(t[1])) for t in (ORDER_NO_A if ja is None else ORDER_FULL).split()]


def _parse(s):
    out = []
    for t in s.split():
        if t[0] == 'a':
            h, r = t[1:].split(':')
            out.append(('a', int(h) // G, (int(h) % G, int(r[0]), int(r[1]))))
        else:
            out.append((t[0], int(t[1:]) // G, int(t[1:]) % G))
    return out


def _plan():
    ramp = [_parse(s) for s in RAMP]
    tail = [('S', 0, (0, NC))]
    for j in range(LOOPS[-1][1], NJ):
        tail += _step_ops(None, j, j - 1)
    lo = 0
    for n in range(NC):
        tail.append(('F', NJ - 1, n))
        if n + 1 in OUT_STARTS:
            tail.append(('S', 1, (lo, n + 1)))
            lo = n + 1
    assert lo == NC - 1

    have = set()

    def need(ops, sem):
        items = []

        def add(key, j, i):
            if (key, j, i) not in have:
                have.add((key, j, i))
                items.append((key, j, i))

        for kind, j, i in ops:
            if kind == 'S':
                continue
            if kind == 'A':
                for t in range(XB):
                    add('x', j // GPB, t)
            if kind == 'a':
                for t in range(i[1], i[2]):
                    add('x', j // GPB, t)
                i = i[0]
            add({'A': 'wq', 'a': 'wq', 'B': 'k', 'P': 'k', 'D': 'v', 'C': 'wo', 'F': 'wo'}[kind], j, i)
        first = {}
        for n, (key, j, i) in enumerate(items):
            first.setdefault((key, j), n)
        items.sort(key=lambda t: (first[(t[0], t[1])], t[2]))
        out = []
        for key, j, i in items:
            if out and out[-1][0] == key and out[-1][1] == j and out[-1][3] == i:
                out[-1][3] = i + 1
            else:
                out.append([key, j, i, i + 1])
        return [(sem, *o) for o in out]

    dma, ramp_waits, loops = [], [], []
    sem = 0
    for ph in ramp:
        ramp_waits.append(need(ph, sem))
        dma += ramp_waits[-1]
        sem += 1
    sem_xb = sem
    sem += 1
    for (j0, j1, unroll, off, pace) in LOOPS:
        n_iter = (j1 - j0) // unroll
        sem0, xb_iter = sem, None
        for it in range(n_iter):
            ops = []
            for u in range(unroll):
                j = j0 + it * unroll + u
                ops += _step_ops(j + LA, j, j - 1)
            for e in need(ops, sem):
                if e[1] == 'x':
                    xb_iter = it
                    dma.append((sem_xb, *e[1:]))
                else:
                    assert e[3] == 0 and e[4] == (NC if e[1] == 'wo' else G)
                    dma.append(e)
            sem += 1
        loops.append((j0, unroll, n_iter, sem0, xb_iter, off, pace))
    tail_waits = need(tail, sem)
    dma += tail_waits
    return ramp, ramp_waits, loops, tail, tail_waits, dma, sem_xb, sem + 1, sem + 2


_RAMP, _RAMP_WAITS, _LOOPS, _TAIL, _TAIL_WAITS, _DMA, _SEM_XB, _SEM_OUT, _NSEM = _plan()


def _interleave_lanes(vals, level, bits):
    while len(vals) > 1:
        vals = [jnp.where(bits[level], vals[2 * t], vals[2 * t + 1]) for t in range(len(vals) // 2)]
        level += 1
    return vals[0]


def _kernel(ax, ak, av, awq, awo, bx, bk, bv, bwq, bwo, out_hbm,
            x_buf, wq_buf, wo_buf, k_buf, v_buf, acc, q0, q1, q2, q3, o0, o1, o2, o3, o_stage,
            zero_ref, sems):
    srcs = ((ax, ak, av, awq, awo), (bx, bk, bv, bwq, bwo))
    q_bufs = (q0, q1, q2, q3)
    o_bufs = (o0, o1, o2, o3)

    def copy(sem, kind, j, lo, hi):
        br, s = divmod(j, GPB) if isinstance(j, int) else (0, 0)
        _, sk, sv, swq, swo = srcs[br]
        if kind == 'x':
            rows = pl.ds(lo * XR, (hi - lo) * XR)
            return pltpu.make_async_copy(srcs[j][0].at[rows, :], x_buf.at[j, rows, pl.ds(0, D)],
                                         sems.at[sem])
        if kind == 'wq':
            return pltpu.make_async_copy(swq.at[:, pl.ds(s * N + lo * DH, (hi - lo) * DH)],
                                         wq_buf.at[j, :, pl.ds(lo * DH, (hi - lo) * DH)], sems.at[sem])
        if kind == 'wo':
            return pltpu.make_async_copy(swo.at[pl.ds(s * N, N), pl.ds(lo * CN, (hi - lo) * CN)],
                                         wo_buf.at[j, :, pl.ds(lo * CN, (hi - lo) * CN)], sems.at[sem])
        src, buf = (sk, k_buf) if kind == 'k' else (sv, v_buf)
        return pltpu.make_async_copy(src.at[:, pl.ds(s * G + lo, hi - lo)],
                                     buf.at[j, :, pl.ds(lo, hi - lo)], sems.at[sem])

    for e in _DMA:
        copy(*e).start()
    acc[...] = jnp.zeros_like(acc)
    zero_ref[...] = jnp.zeros_like(zero_ref)

    out_copies = []

    def start_out(br, r0, rows, lo, hi):
        cp = pltpu.make_async_copy(
            o_stage.at[br, pl.ds(r0, rows), pl.ds(lo * CN, (hi - lo) * CN)],
            out_hbm.at[pl.ds(r0, rows), pl.ds(br * D + lo * CN, (hi - lo) * CN)],
            sems.at[_SEM_OUT])
        cp.start()
        out_copies.append(cp)

    def run_ops(ops, base, first, off, pace, stage_rel=()):
        xs, o_prev, probs, s_off, hist = {}, {}, {}, {}, []
        never = zero_ref[...] != 0
        lane32 = lax.broadcasted_iota(jnp.int32, (SK, 128), 1)
        even = (lane32 & 32) == 0
        low = (lane32 & 64) == 0
        seg = lane32 >> 5
        for kind, jr, i in ops:
            j = base + jr
            if kind == 'A':
                key = j // GPB if isinstance(j, int) else jr
                if key not in xs:
                    xs[key] = x_buf[j // GPB, :, 0:D]
                q_bufs[i][j % NQ] = jnp.dot(xs[key], wq_buf[j, :, i * DH:(i + 1) * DH],
                                            preferred_element_type=F32).astype(BF16)
            elif kind == 'a':
                i, r0, r1 = i[0], i[1] * XR, i[2] * XR
                q_bufs[i][j % NQ, r0:r1, :] = jnp.dot(
                    x_buf[j // GPB, r0:r1, 0:D], wq_buf[j, :, i * DH:(i + 1) * DH],
                    preferred_element_type=F32).astype(BF16)
            elif kind == 'P':
                rb = 128 - off[(jr - first) * G + i]
                tiles = []
                for g in range(NG):
                    blocks = []
                    for bb in range(rb // SK, BG):
                        k0 = max(rb - bb * SK, 0)
                        lane = lax.broadcasted_iota(jnp.int32, (SK - k0, 128), 1)
                        bits = [(lane & (1 << t)) == 0 for t in range(5)]
                        kf = k_buf[j, g * BG + bb, i, k0:SK, :].astype(F32)
                        r0 = g * 128 + bb * SQ
                        qf = q_bufs[i][j % NQ, r0:r0 + SQ, :].astype(F32)
                        parts = []
                        for u in range(SQ // 8):
                            q8 = qf[u * 8:(u + 1) * 8]
                            if len(hist) >= pace:
                                dep = hist[-pace]
                                d8 = dep[0:8]
                                for t in range(1, dep.shape[0] // 8):
                                    d8 = jnp.maximum(d8, dep[t * 8:(t + 1) * 8])
                                q8 = jnp.where(never, d8, q8)
                            cols = [jnp.broadcast_to(
                                jnp.sum(kf * q8[t:t + 1, :], axis=-1, keepdims=True), kf.shape)
                                for t in range(8)]
                            parts.append(_interleave_lanes(cols, 0, bits))
                            hist.append(parts[-1])
                        blocks.append(_interleave_lanes(parts, 3, bits))
                    tiles.append(jnp.concatenate(blocks, axis=0))
                s_off[(jr, i)] = tiles
            elif kind == 'B':
                rb = 128 - off[(jr - first) * G + i]
                st = []
                for g in range(NG):
                    qg = q_bufs[i][j % NQ, g * 128:(g + 1) * 128, :]
                    kg = k_buf[j, g * BG:(g + 1) * BG, i].reshape(128, DH)[:rb]
                    st.append(lax.dot_general(kg, qg, (((1,), (1,)), ((), ())),
                                              preferred_element_type=F32))
                tiles = s_off.pop((jr, i))
                pts = []
                for g in range(NG):
                    full = jnp.concatenate([st[g], tiles[g]], axis=0)
                    blk = [full[bb * SK:(bb + 1) * SK] for bb in range(BG)]
                    s = jnp.where(low, jnp.where(even, blk[0], blk[1]),
                                  jnp.where(even, blk[2], blk[3]))
                    m = jnp.max(s, axis=0, keepdims=True)
                    e = jnp.exp2((s - m) * EXP2_SCALE)
                    l = jnp.sum(e, axis=0, keepdims=True)
                    pts.append(e * pl.reciprocal(l, approx=True))
                probs[(jr, i)] = jnp.concatenate(pts, axis=0).T
            elif kind == 'D':
                p = probs.pop((jr, i))
                for b in range(BG):
                    pb = p[b * SQ:(b + 1) * SQ]
                    lhs = jnp.concatenate([jnp.where(seg == g, pb, 0.0) for g in range(NG)], axis=0)
                    vb = jnp.concatenate([v_buf[j, g * BG + b, i] for g in range(NG)], axis=0)
                    o = jnp.dot(lhs.astype(BF16), vb, preferred_element_type=F32).astype(BF16)
                    for g in range(NG):
                        r0 = (g * BG + b) * SQ
                        o_bufs[i][r0:r0 + SQ, :] = o[g * SQ:(g + 1) * SQ]
            elif kind == 'S':
                start_out(jr, 0, M, *i)
            else:
                if jr not in o_prev:
                    o_prev[jr] = jnp.concatenate([ob[...] for ob in o_bufs], axis=1)
                cols = slice(i * CN, (i + 1) * CN)
                val = acc[j // GPB, :, cols] + jnp.dot(o_prev[jr], wo_buf[j, :, cols],
                                                       preferred_element_type=F32)
                if kind == 'C':
                    acc[j // GPB, :, cols] = val
                    if jr in stage_rel:
                        o_stage[j // GPB, :, cols] = val.astype(BF16)
                elif i < NC - 1:
                    o_stage[1, :, cols] = val.astype(BF16)
                else:
                    rows = M // LAST_SPLIT
                    for s in range(LAST_SPLIT):
                        o_stage[1, s * rows:(s + 1) * rows, cols] = (
                            val[s * rows:(s + 1) * rows].astype(BF16))
                        start_out(1, s * rows, rows, i, i + 1)
        assert not probs and not s_off

    for ph, waits in zip(_RAMP, _RAMP_WAITS):
        for e in waits:
            copy(*e).wait()
        run_ops(ph, 0, 0, OFF_RAMP, PACE)

    for (j0, unroll, n_iter, sem0, xb_iter, off, pace) in _LOOPS:
        ops = []
        for u in range(unroll):
            ops += _step_ops(u + LA, u, u - 1)
        stage_rel = tuple(u - 1 for u in range(unroll)
                          if any(j0 + t * unroll + u - 1 == GPB - 1 for t in range(n_iter)))

        def body(it, carry, j0=j0, unroll=unroll, sem0=sem0, xb_iter=xb_iter, off=off, pace=pace,
                 ops=ops, stage_rel=stage_rel):
            jb = j0 + it * unroll
            if xb_iter is not None:
                @pl.when(it == xb_iter)
                def _():
                    copy(_SEM_XB, 'x', 1, 0, XB).wait()
            for u in range(unroll):
                copy(sem0 + it, 'wq', jb + u + LA, 0, G).wait()
                copy(sem0 + it, 'k', jb + u, 0, G).wait()
                copy(sem0 + it, 'v', jb + u, 0, G).wait()
                copy(sem0 + it, 'wo', jb + u - 1, 0, NC).wait()
            run_ops(ops, jb, 0, off, pace, stage_rel)
            return carry

        lax.fori_loop(0, n_iter, body, 0)

    for e in _TAIL_WAITS:
        copy(*e).wait()
    run_ops(_TAIL, 0, LOOPS[-1][1], OFF_TAIL, PACE)
    for cp in out_copies:
        cp.wait()


def _compiler_params():
    vmem = 100 * 1024 * 1024
    try:
        return pltpu.CompilerParams(vmem_limit_bytes=vmem, disable_semaphore_checks=True)
    except TypeError:
        return pltpu.CompilerParams(vmem_limit_bytes=vmem)


@jax.jit
def pallas_concat_heads__mha_block_cached__mha_block_cached__near_ridge_kernel(
    A_x: jax.Array,
    A_k_cache: jax.Array,
    A_v_cache: jax.Array,
    A_wq: jax.Array,
    A_wo: jax.Array,
    B_x: jax.Array,
    B_k_cache: jax.Array,
    B_v_cache: jax.Array,
    B_wq: jax.Array,
    B_wo: jax.Array,
):
    hbm = pl.BlockSpec(memory_space=pl.ANY)
    out = pl.pallas_call(
        _kernel,
        in_specs=[hbm] * 10,
        out_specs=hbm,
        out_shape=jax.ShapeDtypeStruct((M, 2 * D), BF16),
        scratch_shapes=[
            pltpu.VMEM((2, M, D + PAD), BF16),
            pltpu.VMEM((NJ, D, N + PAD), BF16),
            pltpu.VMEM((NJ, N, D + PAD), BF16),
            pltpu.VMEM((NJ, B, G, SK, DH), BF16),
            pltpu.VMEM((NJ, B, G, SK, DH), BF16),
            pltpu.VMEM((2, M, D), F32),
        ] + [pltpu.VMEM((NQ, M, DH), BF16)] * G
          + [pltpu.VMEM((M, DH), BF16)] * G + [
            pltpu.VMEM((2, M, D), BF16),
            pltpu.VMEM((8, 128), jnp.int32),
            pltpu.SemaphoreType.DMA((_NSEM,)),
        ],
        compiler_params=_compiler_params(),
    )(A_x.reshape(M, D), A_k_cache, A_v_cache, A_wq, A_wo,
      B_x.reshape(M, D), B_k_cache, B_v_cache, B_wq, B_wo)
    return out.reshape(B, SQ, 2 * D)
```

```python
import jax
import jax.numpy as jnp
from jax import lax
import jax.experimental.pallas as pl
import jax.experimental.pallas.tpu as pltpu

B, SQ, D = 16, 32, 1024
H, SK, DH = 32, 32, 128
M = B * SQ
BG = 128 // SQ
NG = B // BG
G = 4
N = G * DH
GPB = H // G
NJ = 2 * GPB
CN = 128
NC = D // CN
NQ = 4
LA = 3
KG = 2
KS = D // 128
PAD = 128
LAST_SPLIT = 8
F32 = jnp.float32
BF16 = jnp.bfloat16
EXP2_SCALE = (DH ** -0.5) * 1.4426950408889634

ORDER_FULL = 'P0 P1 P2 P3 A3 B0 C0 B1 C1 B2 C2 B3 A0 D0 A1 C3 D1 A2 C4 D2 C5 C6 C7 D3'
ORDER_NO_A = 'P0 P1 P2 P3 C0 B0 C1 C2 D0 B1 C3 C4 D1 B2 C5 B3 C6 D2 C7 D3'
RAMP = ['k01', 'k12', 'k23', 'k35', 'k58', 'A8 A9 A10 A11',
        'P0 P1 P2 P3 A12 B0 B1 B2 B3 A13 D0 A14 D1 D2 A15 D3']
N_EARLY_DMA = 55
LATE_DMA_PHASE = 3
LOOPS = ((1, 3, 1, (32, 48, 48, 48), 5),
         (3, 13, 2, (32, 48, 48, 48, 48, 48, 48, 48), 4))
OFF_RAMP = (32, 16, 16, 32)
OFF_TAIL = (16, 32, 32, 16) * 3
PACE = 5
OUT_STARTS = (2, 4, 6, 7)


def _step_ops(ja, jb, jc):
    grp = {'A': ja, 'B': jb, 'D': jb, 'P': jb, 'C': jc}
    return [(t[0], grp[t[0]], int(t[1])) for t in (ORDER_NO_A if ja is None else ORDER_FULL).split()]


def _parse(s):
    return [('k', 0, (int(t[1]), int(t[2]))) if t[0] == 'k' else (t[0], int(t[1:]) // G, int(t[1:]) % G)
            for t in s.split()]


def _plan():
    ramp = [_parse(s) for s in RAMP]
    tail = [('S', 0, (0, NC))]
    for j in range(LOOPS[-1][1], NJ):
        tail += _step_ops(None, j, j - 1)
    lo = 0
    for n in range(NC):
        tail.append(('F', NJ - 1, n))
        if n + 1 in OUT_STARTS:
            tail.append(('S', 1, (lo, n + 1)))
            lo = n + 1
    assert lo == NC - 1

    have = set()

    def need(ops, sem):
        items = []

        def add(key, j, i):
            if (key, j, i) not in have:
                have.add((key, j, i))
                items.append((key, j, i))

        for kind, j, i in ops:
            if kind == 'S':
                continue
            if kind == 'k':
                for t in range(*i):
                    add('xk', 0, t)
                    for jj in range(KG):
                        add('wk', jj, t)
                have.add(('x', 0, 0))
                have.update(('wq', jj, t) for jj in range(KG) for t in range(G))
                continue
            if kind == 'A':
                add('x', j // GPB, 0)
            add({'A': 'wq', 'B': 'k', 'P': 'k', 'D': 'v', 'C': 'wo', 'F': 'wo'}[kind], j, i)
        first = {}
        for n, (key, j, i) in enumerate(items):
            first.setdefault((key, j), n)
        items.sort(key=lambda t: (first[(t[0], t[1])], t[2]))
        out = []
        for key, j, i in items:
            if out and out[-1][0] == key and out[-1][1] == j and out[-1][3] == i:
                out[-1][3] = i + 1
            else:
                out.append([key, j, i, i + 1])
        return [(sem, *o) for o in out]

    dma, ramp_waits, loops = [], [], []
    sem = 0
    for ph in ramp:
        ramp_waits.append(need(ph, sem))
        dma += ramp_waits[-1]
        sem += 1
    sem_xb = sem
    sem += 1
    for (j0, j1, unroll, off, pace) in LOOPS:
        n_iter = (j1 - j0) // unroll
        sem0, xb_iter = sem, None
        for it in range(n_iter):
            ops = []
            for u in range(unroll):
                j = j0 + it * unroll + u
                ops += _step_ops(j + LA, j, j - 1)
            for e in need(ops, sem):
                if e[1] == 'x':
                    xb_iter = it
                    dma.append((sem_xb, *e[1:]))
                else:
                    assert e[3] == 0 and e[4] == (NC if e[1] == 'wo' else G)
                    dma.append(e)
            sem += 1
        loops.append((j0, unroll, n_iter, sem0, xb_iter, off, pace))
    tail_waits = need(tail, sem)
    dma += tail_waits
    return ramp, ramp_waits, loops, tail, tail_waits, dma, sem_xb, sem + 1, sem + 2


_RAMP, _RAMP_WAITS, _LOOPS, _TAIL, _TAIL_WAITS, _DMA, _SEM_XB, _SEM_OUT, _NSEM = _plan()


def _interleave_lanes(vals, level, bits):
    while len(vals) > 1:
        vals = [jnp.where(bits[level], vals[2 * t], vals[2 * t + 1]) for t in range(len(vals) // 2)]
        level += 1
    return vals[0]


def _kernel(ax, ak, av, awq, awo, bx, bk, bv, bwq, bwo, out_hbm,
            x_buf, wq_buf, wo_buf, k_buf, v_buf, acc, q0, q1, q2, q3, o0, o1, o2, o3, o_stage,
            zero_ref, q_acc, sems):
    srcs = ((ax, ak, av, awq, awo), (bx, bk, bv, bwq, bwo))
    q_bufs = (q0, q1, q2, q3)
    o_bufs = (o0, o1, o2, o3)

    def copy(sem, kind, j, lo, hi):
        br, s = divmod(j, GPB) if isinstance(j, int) else (0, 0)
        _, sk, sv, swq, swo = srcs[br]
        if kind == 'x':
            return pltpu.make_async_copy(srcs[j][0], x_buf.at[j, :, pl.ds(0, D)], sems.at[sem])
        if kind == 'xk':
            cols = pl.ds(lo * 128, (hi - lo) * 128)
            return pltpu.make_async_copy(ax.at[:, cols], x_buf.at[0, :, cols], sems.at[sem])
        if kind == 'wk':
            rows = pl.ds(lo * 128, (hi - lo) * 128)
            return pltpu.make_async_copy(awq.at[rows, pl.ds(j * N, N)],
                                         wq_buf.at[j, rows, pl.ds(0, N)], sems.at[sem])
        if kind == 'wq':
            return pltpu.make_async_copy(swq.at[:, pl.ds(s * N + lo * DH, (hi - lo) * DH)],
                                         wq_buf.at[j, :, pl.ds(lo * DH, (hi - lo) * DH)], sems.at[sem])
        if kind == 'wo':
            return pltpu.make_async_copy(swo.at[pl.ds(s * N, N), pl.ds(lo * CN, (hi - lo) * CN)],
                                         wo_buf.at[j, :, pl.ds(lo * CN, (hi - lo) * CN)], sems.at[sem])
        src, buf = (sk, k_buf) if kind == 'k' else (sv, v_buf)
        return pltpu.make_async_copy(src.at[:, pl.ds(s * G + lo, hi - lo)],
                                     buf.at[j, :, pl.ds(lo, hi - lo)], sems.at[sem])

    for e in _DMA[:N_EARLY_DMA]:
        copy(*e).start()
    acc[...] = jnp.zeros_like(acc)
    zero_ref[...] = jnp.zeros_like(zero_ref)

    out_copies = []

    def start_out(br, r0, rows, lo, hi):
        cp = pltpu.make_async_copy(
            o_stage.at[br, pl.ds(r0, rows), pl.ds(lo * CN, (hi - lo) * CN)],
            out_hbm.at[pl.ds(r0, rows), pl.ds(br * D + lo * CN, (hi - lo) * CN)],
            sems.at[_SEM_OUT])
        cp.start()
        out_copies.append(cp)

    def run_ops(ops, base, first, off, pace, stage_rel=()):
        xs, o_prev, probs, s_off, hist = {}, {}, {}, {}, []
        never = zero_ref[...] != 0
        lane32 = lax.broadcasted_iota(jnp.int32, (SK, 128), 1)
        even = (lane32 & 32) == 0
        low = (lane32 & 64) == 0
        seg = lane32 >> 5
        for kind, jr, i in ops:
            j = base + jr
            if kind == 'A':
                key = j // GPB if isinstance(j, int) else jr
                if key not in xs:
                    xs[key] = x_buf[j // GPB, :, 0:D]
                q_bufs[i][j % NQ] = jnp.dot(xs[key], wq_buf[j, :, i * DH:(i + 1) * DH],
                                            preferred_element_type=F32).astype(BF16)
            elif kind == 'k':
                for jj in range(KG):
                    r = None
                    for t in range(*i):
                        ks = slice(t * 128, (t + 1) * 128)
                        d = jnp.dot(x_buf[0, :, ks], wq_buf[jj, ks, 0:N], preferred_element_type=F32)
                        r = d if r is None else r + d
                    if i[0] > 0:
                        r = r + q_acc[jj]
                    if i[1] < KS:
                        q_acc[jj] = r
                    else:
                        for h in range(G):
                            q_bufs[h][jj] = r[:, h * DH:(h + 1) * DH].astype(BF16)
            elif kind == 'P':
                rb = 128 - off[(jr - first) * G + i]
                tiles = []
                for g in range(NG):
                    blocks = []
                    for bb in range(rb // SK, BG):
                        k0 = max(rb - bb * SK, 0)
                        lane = lax.broadcasted_iota(jnp.int32, (SK - k0, 128), 1)
                        bits = [(lane & (1 << t)) == 0 for t in range(5)]
                        kf = k_buf[j, g * BG + bb, i, k0:SK, :].astype(F32)
                        r0 = g * 128 + bb * SQ
                        qf = q_bufs[i][j % NQ, r0:r0 + SQ, :].astype(F32)
                        parts = []
                        for u in range(SQ // 8):
                            q8 = qf[u * 8:(u + 1) * 8]
                            if len(hist) >= pace:
                                dep = hist[-pace]
                                d8 = dep[0:8]
                                for t in range(1, dep.shape[0] // 8):
                                    d8 = jnp.maximum(d8, dep[t * 8:(t + 1) * 8])
                                q8 = jnp.where(never, d8, q8)
                            cols = [jnp.broadcast_to(
                                jnp.sum(kf * q8[t:t + 1, :], axis=-1, keepdims=True), kf.shape)
                                for t in range(8)]
                            parts.append(_interleave_lanes(cols, 0, bits))
                            hist.append(parts[-1])
                        blocks.append(_interleave_lanes(parts, 3, bits))
                    tiles.append(jnp.concatenate(blocks, axis=0))
                s_off[(jr, i)] = tiles
            elif kind == 'B':
                rb = 128 - off[(jr - first) * G + i]
                st = []
                for g in range(NG):
                    qg = q_bufs[i][j % NQ, g * 128:(g + 1) * 128, :]
                    kg = k_buf[j, g * BG:(g + 1) * BG, i].reshape(128, DH)[:rb]
                    st.append(lax.dot_general(kg, qg, (((1,), (1,)), ((), ())),
                                              preferred_element_type=F32))
                tiles = s_off.pop((jr, i))
                pts = []
                for g in range(NG):
                    full = jnp.concatenate([st[g], tiles[g]], axis=0)
                    blk = [full[bb * SK:(bb + 1) * SK] for bb in range(BG)]
                    s = jnp.where(low, jnp.where(even, blk[0], blk[1]),
                                  jnp.where(even, blk[2], blk[3]))
                    m = jnp.max(s, axis=0, keepdims=True)
                    e = jnp.exp2((s - m) * EXP2_SCALE)
                    l = jnp.sum(e, axis=0, keepdims=True)
                    pts.append(e * (1.0 / l))
                probs[(jr, i)] = jnp.concatenate(pts, axis=0).T
            elif kind == 'D':
                p = probs.pop((jr, i))
                for b in range(BG):
                    pb = p[b * SQ:(b + 1) * SQ]
                    lhs = jnp.concatenate([jnp.where(seg == g, pb, 0.0) for g in range(NG)], axis=0)
                    vb = jnp.concatenate([v_buf[j, g * BG + b, i] for g in range(NG)], axis=0)
                    o = jnp.dot(lhs.astype(BF16), vb, preferred_element_type=F32).astype(BF16)
                    for g in range(NG):
                        r0 = (g * BG + b) * SQ
                        o_bufs[i][r0:r0 + SQ, :] = o[g * SQ:(g + 1) * SQ]
            elif kind == 'S':
                start_out(jr, 0, M, *i)
            else:
                if jr not in o_prev:
                    o_prev[jr] = jnp.concatenate([ob[...] for ob in o_bufs], axis=1)
                cols = slice(i * CN, (i + 1) * CN)
                val = acc[j // GPB, :, cols] + jnp.dot(o_prev[jr], wo_buf[j, :, cols],
                                                       preferred_element_type=F32)
                if kind == 'C':
                    acc[j // GPB, :, cols] = val
                    if jr in stage_rel:
                        o_stage[j // GPB, :, cols] = val.astype(BF16)
                elif i < NC - 1:
                    o_stage[1, :, cols] = val.astype(BF16)
                else:
                    rows = M // LAST_SPLIT
                    for s in range(LAST_SPLIT):
                        o_stage[1, s * rows:(s + 1) * rows, cols] = (
                            val[s * rows:(s + 1) * rows].astype(BF16))
                        start_out(1, s * rows, rows, i, i + 1)
        assert not probs and not s_off

    for n, (ph, waits) in enumerate(zip(_RAMP, _RAMP_WAITS)):
        for e in waits:
            copy(*e).wait()
        run_ops(ph, 0, 0, OFF_RAMP, PACE)
        if n == LATE_DMA_PHASE:
            for e in _DMA[N_EARLY_DMA:]:
                copy(*e).start()

    for (j0, unroll, n_iter, sem0, xb_iter, off, pace) in _LOOPS:
        ops = []
        for u in range(unroll):
            ops += _step_ops(u + LA, u, u - 1)
        stage_rel = tuple(u - 1 for u in range(unroll)
                          if any(j0 + t * unroll + u - 1 == GPB - 1 for t in range(n_iter)))

        def body(it, carry, j0=j0, unroll=unroll, sem0=sem0, xb_iter=xb_iter, off=off, pace=pace,
                 ops=ops, stage_rel=stage_rel):
            jb = j0 + it * unroll
            if xb_iter is not None:
                @pl.when(it == xb_iter)
                def _():
                    copy(_SEM_XB, 'x', 1, 0, 1).wait()
            for u in range(unroll):
                copy(sem0 + it, 'wq', jb + u + LA, 0, G).wait()
                copy(sem0 + it, 'k', jb + u, 0, G).wait()
                copy(sem0 + it, 'v', jb + u, 0, G).wait()
                copy(sem0 + it, 'wo', jb + u - 1, 0, NC).wait()
            run_ops(ops, jb, 0, off, pace, stage_rel)
            return carry

        lax.fori_loop(0, n_iter, body, 0)

    for e in _TAIL_WAITS:
        copy(*e).wait()
    run_ops(_TAIL, 0, LOOPS[-1][1], OFF_TAIL, PACE)
    for cp in out_copies:
        cp.wait()


def _compiler_params():
    vmem = 100 * 1024 * 1024
    try:
        return pltpu.CompilerParams(vmem_limit_bytes=vmem, disable_semaphore_checks=True)
    except TypeError:
        return pltpu.CompilerParams(vmem_limit_bytes=vmem)


@jax.jit
def pallas_concat_heads__mha_block_cached__mha_block_cached__near_ridge_kernel(
    A_x: jax.Array,
    A_k_cache: jax.Array,
    A_v_cache: jax.Array,
    A_wq: jax.Array,
    A_wo: jax.Array,
    B_x: jax.Array,
    B_k_cache: jax.Array,
    B_v_cache: jax.Array,
    B_wq: jax.Array,
    B_wo: jax.Array,
):
    hbm = pl.BlockSpec(memory_space=pl.ANY)
    out = pl.pallas_call(
        _kernel,
        in_specs=[hbm] * 10,
        out_specs=hbm,
        out_shape=jax.ShapeDtypeStruct((M, 2 * D), BF16),
        scratch_shapes=[
            pltpu.VMEM((2, M, D + PAD), BF16),
            pltpu.VMEM((NJ, D, N + PAD), BF16),
            pltpu.VMEM((NJ, N, D + PAD), BF16),
            pltpu.VMEM((NJ, B, G, SK, DH), BF16),
            pltpu.VMEM((NJ, B, G, SK, DH), BF16),
            pltpu.VMEM((2, M, D), F32),
        ] + [pltpu.VMEM((NQ, M, DH), BF16)] * G
          + [pltpu.VMEM((M, DH), BF16)] * G + [
            pltpu.VMEM((2, M, D), BF16),
            pltpu.VMEM((8, 128), jnp.int32),
            pltpu.VMEM((KG, M, N), F32),
            pltpu.SemaphoreType.DMA((_NSEM,)),
        ],
        compiler_params=_compiler_params(),
    )(A_x.reshape(M, D), A_k_cache, A_v_cache, A_wq, A_wo,
      B_x.reshape(M, D), B_k_cache, B_v_cache, B_wq, B_wo)
    return out.reshape(B, SQ, 2 * D)
```
